```python
import jax
import jax.numpy as jnp

def _softmax(x, axis=-1):
    return jax.nn.softmax(x, axis=axis)
def _gelu(x):
    return jax.nn.gelu(x, approximate=True)
def _silu(x):
    return jax.nn.silu(x)
def _sigmoid(x):
    return jax.nn.sigmoid(x)
def _layernorm(x, axis=-1, eps=1e-5):
    m = jnp.mean(x, axis=axis, keepdims=True)
    v = jnp.var(x, axis=axis, keepdims=True)
    return (x - m) / jnp.sqrt(v + eps)
def _scatter_add(tgt, idx, src, axis=0):
    return tgt.at[idx].add(src)
def _segment_sum(src, seg, n):
    return jax.ops.segment_sum(src, seg, n)
class _Rng:
    def __init__(self, key):
        self._k = key
    def _next(self):
        self._k, sub = jax.random.split(self._k)
        return sub
    def normal(self, shape):
        return jax.random.normal(self._next(), shape, dtype=jnp.bfloat16)
    def randint(self, lo, hi, shape):
        return jax.random.randint(self._next(), shape, lo, hi, dtype=jnp.int32)
    def uniform(self, shape, lo=0.0, hi=1.0):
        return jax.random.uniform(self._next(), shape, jnp.bfloat16, lo, hi)
    def permutation(self, n):
        return jax.random.permutation(self._next(), n)


kernel_name = 'standalone__winograd__vision'

def setup_inputs():
    _rng = _Rng(jax.random.key(int.from_bytes(__import__("os").urandom(4), "little")))
    _w = (lambda a: (lambda t: t.astype(jnp.bfloat16) if jnp.issubdtype(t.dtype, jnp.floating) else t)(jnp.asarray(a)))
    H = W = 512 // 2 * 2
    C = 192
    return {
        "x": _w((lambda *s: _rng.normal(s) * 0.05)(1, H, W, C)),
        "w": _w((lambda *s: _rng.normal(s) * 0.05)(3, 3, C, C)),
    }

def reference(x, w):
    N, H, W, C = x.shape
    K = w.shape[-1]
    G  = jnp.array([[1.0,0.0,0.0],[0.5,0.5,0.5],[0.5,-0.5,0.5],[0.0,0.0,1.0]], dtype=x.dtype)
    Bt = jnp.array([[1.0,0.0,-1.0,0.0],[0.0,1.0,1.0,0.0],[0.0,-1.0,1.0,0.0],[0.0,1.0,0.0,-1.0]], dtype=x.dtype)
    At = jnp.array([[1.0,1.0,1.0,0.0],[0.0,1.0,-1.0,-1.0]], dtype=x.dtype)
    U = jnp.einsum("ar,rsck,bs->abck", G, w, G)
    xp = jnp.pad(x, ((0,0),(1,1),(1,1),(0,0)))
    nH, nW = H // 2, W // 2
    patches = []
    for i in range(4):
        for j in range(4):
            patches.append(xp[:, i:i + 2 * nH:2, j:j + 2 * nW:2, :])
    d = jnp.stack(patches).reshape(4, 4, N * nH * nW, C)
    V = jnp.einsum("ai,ijpc,bj->abpc", Bt, d, Bt)
    M = jnp.einsum("abck,abpc->abpk", U, V)
    Y = jnp.einsum("ma,abpk,nb->pmnk", At, M, At)
    Y = Y.reshape(N, nH, nW, 2, 2, K)
    Y = (lambda x, *d: x.transpose(*d))(Y, 0, 1, 3, 2, 4, 5).reshape(N, H, W, K)
    return Y
```

```python
import jax
import jax.numpy as jnp
import jax.experimental.pallas as pl
import jax.experimental.pallas.tpu as pltpu

R = 16
BF, F32 = jnp.bfloat16, jnp.float32


def _kernel(x_ref, top_ref, bot_ref, w_ref, o_ref, u_ref, v_ref):
    i = pl.program_id(0)
    n = pl.num_programs(0)
    C, W = x_ref.shape[1:]

    @pl.when(i == 0)
    def _():
        g0, g1, g2 = (w_ref[k].astype(F32) for k in range(3))
        s = g0 + g2
        t = g0 * (1 / 24) + g2 * (1 / 6)
        u_ref[0] = (g0 * 0.25).astype(BF)
        u_ref[1] = ((s + g1) * (-1 / 6)).astype(BF)
        u_ref[2] = ((s - g1) * (-1 / 6)).astype(BF)
        u_ref[3] = (t + g1 * (1 / 12)).astype(BF)
        u_ref[4] = (t - g1 * (1 / 12)).astype(BF)
        u_ref[5] = g2.astype(BF)

    lane = jax.lax.broadcasted_iota(jnp.int32, (C // 2, W), 1)
    first, last = lane == 0, lane == W - 1
    zero = jnp.zeros((C // 2, W), jnp.uint32)

    def row(r):
        if r < 0:
            return jnp.where(i > 0, top_ref[0].astype(F32), 0.0)
        if r >= R:
            return jnp.where(i < n - 1, bot_ref[0].astype(F32), 0.0)
        return x_ref[r].astype(F32)

    for t in range(R // 4):
        d0, d1, d2, d3, d4, d5 = (row(4 * t - 1 + k) for k in range(6))
        p, q = d4 - 4 * d2, d3 - 4 * d1
        r, s = d4 - d2, 2 * (d3 - d1)
        vs = (4 * d0 - 5 * d2 + d4, p + q, p - q, r + s, r - s,
              4 * d1 - 5 * d3 + d5)
        m = []
        for a, v in enumerate(vs):
            v = v.astype(BF)
            b = pltpu.bitcast(v, jnp.uint32)
            v_ref[a, 0:C] = pltpu.bitcast(
                jnp.where(first, zero, pltpu.roll(b, 1, 1)), BF)
            v_ref[a, C:2 * C] = v
            v_ref[a, 2 * C:3 * C] = pltpu.bitcast(
                jnp.where(last, zero, pltpu.roll(b, W - 1, 1)), BF)
            m.append(jnp.dot(u_ref[a], v_ref[a], preferred_element_type=F32))
        p, q = m[1] + m[2], m[1] - m[2]
        r, s = m[3] + m[4], m[3] - m[4]
        o_ref[4 * t] = (m[0] + p + r).astype(BF)
        o_ref[4 * t + 1] = (q + 2 * s).astype(BF)
        o_ref[4 * t + 2] = (p + 4 * r).astype(BF)
        o_ref[4 * t + 3] = (q + 8 * s + m[5]).astype(BF)


@jax.jit
def pallas_standalone__winograd__vision_kernel(x, w):
    _, H, W, C = x.shape
    K = w.shape[-1]
    xt = x[0].transpose(0, 2, 1)
    wt = w.reshape(3, 3 * C, K).transpose(0, 2, 1)
    out = pl.pallas_call(
        _kernel,
        grid=(H // R,),
        in_specs=[
            pl.BlockSpec((R, C, W), lambda i: (i, 0, 0)),
            pl.BlockSpec((1, C, W), lambda i: (jnp.maximum(i * R - 1, 0), 0, 0)),
            pl.BlockSpec((1, C, W), lambda i: (jnp.minimum(i * R + R, H - 1), 0, 0)),
            pl.BlockSpec((3, K, 3 * C), lambda i: (0, 0, 0)),
        ],
        out_specs=pl.BlockSpec((R, K, W), lambda i: (i, 0, 0)),
        out_shape=jax.ShapeDtypeStruct((H, K, W), x.dtype),
        scratch_shapes=[pltpu.VMEM((6, K, 3 * C), BF), pltpu.VMEM((6, 3 * C, W), BF)],
        compiler_params=pltpu.CompilerParams(
            dimension_semantics=("arbitrary",), vmem_limit_bytes=100 << 20),
    )(xt, xt, xt, wt)
    return out.transpose(0, 2, 1)[None]
```

```python
import jax
import jax.numpy as jnp
import jax.experimental.pallas as pl
import jax.experimental.pallas.tpu as pltpu

R = 16
CC = 16
WC = 512
BF, F32 = jnp.bfloat16, jnp.float32


def _kernel(x_ref, top_ref, bot_ref, w_ref, o_ref, u_ref, v_ref):
    i = pl.program_id(0)
    n = pl.num_programs(0)
    C, W = x_ref.shape[1:]

    @pl.when(i == 0)
    def _():
        g0, g1, g2 = (w_ref[k].astype(F32) for k in range(3))
        s = g0 + g2
        t = g0 * (1 / 24) + g2 * (1 / 6)
        u_ref[0] = (g0 * 0.25).astype(BF)
        u_ref[1] = ((s + g1) * (-1 / 6)).astype(BF)
        u_ref[2] = ((s - g1) * (-1 / 6)).astype(BF)
        u_ref[3] = (t + g1 * (1 / 12)).astype(BF)
        u_ref[4] = (t - g1 * (1 / 12)).astype(BF)
        u_ref[5] = g2.astype(BF)

    lane = jax.lax.broadcasted_iota(jnp.int32, (CC // 2, W), 1)
    first, last = lane == 0, lane == W - 1
    zero = jnp.zeros((CC // 2, W), jnp.uint32)

    def row(r, c):
        if r < 0:
            return jnp.where(i > 0, top_ref[0, c:c + CC].astype(F32), 0.0)
        if r >= R:
            return jnp.where(i < n - 1, bot_ref[0, c:c + CC].astype(F32), 0.0)
        return x_ref[r, c:c + CC].astype(F32)

    def prep(t):
      for c in range(0, C, CC):
        d0, d1, d2, d3, d4, d5 = (row(4 * t - 1 + k, c) for k in range(6))
        p, q = d4 - 4 * d2, d3 - 4 * d1
        r, s = d4 - d2, 2 * (d3 - d1)
        vs = (4 * (d0 - d2) + r, p + q, p - q, r + s, r - s,
              (d5 - d3) - 2 * s)
        for a, v in enumerate(vs):
            v = v.astype(BF)
            b = pltpu.bitcast(v, jnp.uint32)
            v_ref[t % 2, a, c:c + CC] = pltpu.bitcast(
                jnp.where(first, zero, pltpu.roll(b, 1, 1)), BF)
            v_ref[t % 2, a, C + c:C + c + CC] = v
            v_ref[t % 2, a, 2 * C + c:2 * C + c + CC] = pltpu.bitcast(
                jnp.where(last, zero, pltpu.roll(b, W - 1, 1)), BF)

    prep(0)
    for t in range(R // 4):
      if t + 1 < R // 4:
        prep(t + 1)
      for j in range(0, W, WC):
        m = [jnp.dot(u_ref[a], v_ref[t % 2, a, :, j:j + WC],
                     preferred_element_type=F32) for a in range(6)]
        p, q = m[1] + m[2], m[1] - m[2]
        r, s = m[3] + m[4], m[3] - m[4]
        o_ref[4 * t, :, j:j + WC] = (m[0] + p + r).astype(BF)
        o_ref[4 * t + 1, :, j:j + WC] = (q + 2 * s).astype(BF)
        o_ref[4 * t + 2, :, j:j + WC] = (p + 4 * r).astype(BF)
        o_ref[4 * t + 3, :, j:j + WC] = (q + 8 * s + m[5]).astype(BF)


@jax.jit
def pallas_standalone__winograd__vision_kernel(x, w):
    _, H, W, C = x.shape
    K = w.shape[-1]
    xt = x[0].transpose(0, 2, 1)
    wt = w.reshape(3, 3 * C, K).transpose(0, 2, 1)
    out = pl.pallas_call(
        _kernel,
        grid=(H // R,),
        in_specs=[
            pl.BlockSpec((R, C, W), lambda i: (i, 0, 0)),
            pl.BlockSpec((1, C, W), lambda i: (jnp.maximum(i * R - 1, 0), 0, 0)),
            pl.BlockSpec((1, C, W), lambda i: (jnp.minimum(i * R + R, H - 1), 0, 0)),
            pl.BlockSpec((3, K, 3 * C), lambda i: (0, 0, 0)),
        ],
        out_specs=pl.BlockSpec((R, K, W), lambda i: (i, 0, 0)),
        out_shape=jax.ShapeDtypeStruct((H, K, W), x.dtype),
        scratch_shapes=[pltpu.VMEM((6, K, 3 * C), BF), pltpu.VMEM((2, 6, 3 * C, W), BF)],
        compiler_params=pltpu.CompilerParams(
            dimension_semantics=("arbitrary",), vmem_limit_bytes=100 << 20),
    )(xt, xt, xt, wt)
    return out.transpose(0, 2, 1)[None]
```

```python
import jax
import jax.numpy as jnp
import jax.experimental.pallas as pl
import jax.experimental.pallas.tpu as pltpu

T = 6
NI = 4
NO = 2
CC = 16
SIDE = (2, 2, 2, 2, 2, 1, 1, 0)
BF, F32 = jnp.bfloat16, jnp.float32


def _kernel(x_hbm, w_ref, o_hbm, xb, ob, u_ref, va, vb, isem, osem):
    H, C, W = x_hbm.shape
    nt = pl.cdiv(H, T)
    tail_o = H - T * (nt - 1)
    tail_i = tail_o - 1

    def in_copy(c, n=T):
        return pltpu.make_async_copy(
            x_hbm.at[pl.ds(T * c + 1, n)], xb.at[c % NI, pl.ds(0, n)],
            isem.at[c % NI])

    def out_copy(t, n=T):
        return pltpu.make_async_copy(
            ob.at[t % NO, pl.ds(0, n)], o_hbm.at[pl.ds(T * t, n)],
            osem.at[t % NO])

    first_row = pltpu.make_async_copy(
        x_hbm.at[pl.ds(0, 1)], xb.at[NI - 1, pl.ds(T - 1, 1)], isem.at[NI - 1])
    first_row.start()
    for c in range(NI - 1):
        in_copy(c).start()
    xb[NI - 1, T - 2] = jnp.zeros((C, W), BF)

    for k in range(0, C, 16):
        ks = slice(k, k + 16)
        g0, g1, g2 = (w_ref[j, ks].astype(F32) for j in range(3))
        u_ref[0, ks] = w_ref[0, ks]
        u_ref[7, ks] = w_ref[2, ks]
        for a, (c0, c1, c2) in ((1, (-2 / 9, -2 / 9, -2 / 9)),
                                (3, (1 / 90, 1 / 45, 2 / 45)),
                                (5, (32 / 45, 16 / 45, 8 / 45))):
            e, o = g0 * c0 + g2 * c2, g1 * c1
            u_ref[a, ks] = (e + o).astype(BF)
            u_ref[a + 1, ks] = (e - o).astype(BF)

    lane = jax.lax.broadcasted_iota(jnp.int32, (CC // 2, W), 1)
    first, last = lane == 0, lane == W - 1
    zero = jnp.zeros((CC // 2, W), jnp.uint32)

    def prep(t, v_ref):
        prev, cur = (t + NI - 1) % NI, t % NI
        for c in range(0, C, CC):
            d0, d1 = (xb[prev, T - 2 + k, c:c + CC].astype(F32) for k in range(2))
            d2, d3, d4, d5, d6, d7 = (
                xb[cur, k, c:c + CC].astype(F32) for k in range(T))

            def put(a, v):
                v = v.astype(BF)
                b = pltpu.bitcast(v, jnp.uint32)
                v_ref[a, c:c + CC] = pltpu.bitcast(
                    jnp.where(first, zero, pltpu.roll(b, 1, 1)), BF)
                v_ref[a, C + c:C + c + CC] = v
                v_ref[a, 2 * C + c:2 * C + c + CC] = pltpu.bitcast(
                    jnp.where(last, zero, pltpu.roll(b, W - 1, 1)), BF)

            put(0, (d0 - d6) + 5.25 * (d4 - d2))
            put(7, (d7 - d1) + 5.25 * (d3 - d5))
            e, o = d2 + d6 - 4.25 * d4, d1 + d5 - 4.25 * d3
            put(1, e + o)
            put(2, e - o)
            h = 2.5 * d3
            e, o = d6 + 0.25 * d2 - 1.25 * d4, 0.5 * d1 - h + 2 * d5
            put(3, e + o)
            put(4, e - o)
            e, o = d6 + 4 * d2 - 5 * d4, 2 * d1 - h + 0.5 * d5
            put(5, e + o)
            put(6, e - o)
            yield

    def matmul(t, v_ref, side=iter(())):
        os_ = t % NO

        def m(a):
            r = jnp.dot(u_ref[a], v_ref[a], preferred_element_type=F32)
            for _ in range(SIDE[a]):
                next(side, None)
            return r

        pq = []
        for a in (1, 3, 5):
            m1, m2 = m(a), m(a + 1)
            pq += [m1 + m2, m1 - m2]
        p1, q1, p3, q3, p5, q5 = pq
        ob[os_, 1] = (q1 + 2 * q3 + 0.5 * q5).astype(BF)
        ob[os_, 2] = (p1 + 4 * p3 + 0.25 * p5).astype(BF)
        ob[os_, 3] = (q1 + 8 * q3 + 0.125 * q5).astype(BF)
        ob[os_, 4] = (p1 + 16 * p3 + 0.0625 * p5).astype(BF)
        y0, y5 = p1 + p3 + p5, q1 + 32 * q3 + 0.03125 * q5
        ob[os_, 0] = (y0 + m(0)).astype(BF)
        ob[os_, 5] = (y5 + m(7)).astype(BF)

    first_row.wait()
    in_copy(0).wait()
    for _ in prep(0, va):
        pass

    def step(t, v_cur, v_next):
        @pl.when(t + 1 < nt - 1)
        def _():
            in_copy(t + 1).wait()

        @pl.when(t + 1 == nt - 1)
        def _():
            in_copy(t + 1, tail_i).wait()

        @pl.when(t + NI - 1 < nt - 1)
        def _():
            in_copy(t + NI - 1).start()

        @pl.when(t + NI - 1 == nt - 1)
        def _():
            s = (nt - 1) % NI
            xb[s, tail_i:T] = jnp.zeros((T - tail_i, C, W), BF)
            in_copy(nt - 1, tail_i).start()

        @pl.when(t >= NO)
        def _():
            out_copy(t - NO).wait()

        matmul(t, v_cur, prep(t + 1, v_next))
        out_copy(t).start()

    def body(j, carry):
        step(2 * j, va, vb)

        @pl.when(2 * j + 1 < nt - 1)
        def _():
            step(2 * j + 1, vb, va)
        return carry

    jax.lax.fori_loop(0, nt // 2, body, 0)
    out_copy(nt - 1 - NO).wait()
    matmul(nt - 1, (va, vb)[(nt - 1) % 2])
    out_copy(nt - 1, tail_o).start()
    for t in range(nt - NO, nt - 1):
        out_copy(t).wait()
    out_copy(nt - 1, tail_o).wait()


@jax.jit
def pallas_standalone__winograd__vision_kernel(x, w):
    _, H, W, C = x.shape
    K = w.shape[-1]
    xt = x[0].transpose(0, 2, 1)
    wt = w.reshape(3, 3 * C, K).transpose(0, 2, 1)
    out = pl.pallas_call(
        _kernel,
        in_specs=[pl.BlockSpec(memory_space=pl.ANY),
                  pl.BlockSpec(memory_space=pltpu.VMEM)],
        out_specs=pl.BlockSpec(memory_space=pl.ANY),
        out_shape=jax.ShapeDtypeStruct((H, K, W), x.dtype),
        scratch_shapes=[
            pltpu.VMEM((NI, T, C, W), BF), pltpu.VMEM((NO, T, K, W), BF),
            pltpu.VMEM((T + 2, K, 3 * C), BF),
            pltpu.VMEM((T + 2, 3 * C, W), BF), pltpu.VMEM((T + 2, 3 * C, W), BF),
            pltpu.SemaphoreType.DMA((NI,)), pltpu.SemaphoreType.DMA((NO,))],
        compiler_params=pltpu.CompilerParams(
            vmem_limit_bytes=100 << 20,
            flags={"XLA_TPU_EVENLY_DISTRIBUTE_CRITICAL_NODES": True}),
    )(xt, wt)
    return out.transpose(0, 2, 1)[None]
```
